```python
import os as _os
_os.environ.setdefault("JAX_PLATFORMS", "cpu")
import jax
import jax.numpy as jnp

def _softmax(x, axis=-1):
    return jax.nn.softmax(x, axis=axis)
def _gelu(x):
    return jax.nn.gelu(x, approximate=True)
def _silu(x):
    return jax.nn.silu(x)
def _sigmoid(x):
    return jax.nn.sigmoid(x)
def _layernorm(x, axis=-1, eps=1e-5):
    m = jnp.mean(x, axis=axis, keepdims=True)
    v = jnp.var(x, axis=axis, keepdims=True)
    return (x - m) / jnp.sqrt(v + eps)
def _scatter_add(tgt, idx, src, axis=0):
    return tgt.at[idx].add(src)
def _segment_sum(src, seg, n):
    return jax.ops.segment_sum(src, seg, n)
class _Rng:
    def __init__(self, key):
        self._k = key
    def _next(self):
        self._k, sub = jax.random.split(self._k)
        return sub
    def normal(self, shape):
        return jax.random.normal(self._next(), shape, dtype=jnp.bfloat16)
    def randint(self, lo, hi, shape):
        return jax.random.randint(self._next(), shape, lo, hi, dtype=jnp.int32)
    def uniform(self, shape, lo=0.0, hi=1.0):
        return jax.random.uniform(self._next(), shape, jnp.bfloat16, lo, hi)
    def permutation(self, n):
        return jax.random.permutation(self._next(), n)


kernel_name = 'parallel_sum__ssm_conv_s5__geglu_ffn__prompt'

def setup_inputs():
    _rng = _Rng(jax.random.key(int.from_bytes(__import__("os").urandom(4), "little")))
    _w = (lambda a: (lambda t: t.astype(jnp.bfloat16) if jnp.issubdtype(t.dtype, jnp.floating) else t)(jnp.asarray(a)))
    def _A_setup():
        B, S, D = 1, 2048, 512
        P = D
        Lambda_re = -0.5 * jnp.exp((lambda *s: _rng.normal(s) * 0.8)(P))
        Lambda_im = (lambda *s: _rng.normal(s) * 0.8)(P) * 1.0
        B_re = (lambda *s: _rng.normal(s) * 0.8)(P, D) * (D ** -0.5)
        B_im = (lambda *s: _rng.normal(s) * 0.8)(P, D) * (D ** -0.5)
        C_re = (lambda *s: _rng.normal(s) * 0.8)(D, P) * (P ** -0.5)
        C_im = (lambda *s: _rng.normal(s) * 0.8)(D, P) * (P ** -0.5)
        log_dt = (lambda *s: _rng.normal(s) * 0.8)(P) * 0.3 - 2.0
        Dskip = (lambda *s: _rng.normal(s) * 0.8)(D)
        return {
            "x": _w((lambda *s: _rng.normal(s) * 0.05)(B, S, D)),
            "Lambda_re": _w(Lambda_re),
            "Lambda_im": _w(Lambda_im),
            "B_re": _w(B_re),
            "B_im": _w(B_im),
            "C_re": _w(C_re),
            "C_im": _w(C_im),
            "log_dt": _w(log_dt),
            "Dskip": _w(Dskip),
        }
    _A_in = _A_setup()

    def _B_setup():
        B, S, D, F = 1, 2048, 512, 1376
        return {
            "x": _w((lambda *s: _rng.normal(s) * 0.05)(B, S, D)),
            "w_gate": _w((lambda *s: _rng.normal(s) * 0.05)(D, F)),
            "w_up": _w((lambda *s: _rng.normal(s) * 0.05)(D, F)),
            "w_down": _w((lambda *s: _rng.normal(s) * 0.05)(F, D)),
        }
    _B_in = _B_setup()

    return {
        "A_x": _A_in["x"],
        "A_Lambda_re": _A_in["Lambda_re"],
        "A_Lambda_im": _A_in["Lambda_im"],
        "A_B_re": _A_in["B_re"],
        "A_B_im": _A_in["B_im"],
        "A_C_re": _A_in["C_re"],
        "A_C_im": _A_in["C_im"],
        "A_log_dt": _A_in["log_dt"],
        "A_Dskip": _A_in["Dskip"],
        "B_x": _B_in["x"],
        "B_w_gate": _B_in["w_gate"],
        "B_w_up": _B_in["w_up"],
        "B_w_down": _B_in["w_down"],
    }

def reference(A_x, A_Lambda_re, A_Lambda_im, A_B_re, A_B_im, A_C_re, A_C_im, A_log_dt, A_Dskip, B_x, B_w_gate, B_w_up, B_w_down):
    def _A_ref(x, Lambda_re, Lambda_im, B_re, B_im, C_re, C_im, log_dt, Dskip):
        Bsz, L, H = x.shape
        Lam = Lambda_re + 1j * Lambda_im
        Bmat = B_re + 1j * B_im
        Cmat = C_re + 1j * C_im
        dt = jnp.exp(log_dt)
        Lam_bar = jnp.exp(dt * Lam)
        B_bar = ((Lam_bar - 1.0) / Lam)[:, None] * Bmat
        Bu = jnp.einsum("bld,pd->blp", x + 0j, B_bar)
        h = jnp.zeros_like(Bu[:, 0, :])
        hs = []
        for t in range(L):
            h = Lam_bar[None, :] * h + Bu[:, t, :]
            hs.append(h)
        hseq = jnp.stack(hs, 1)
        y = 2.0 * jnp.einsum("blp,dp->bld", hseq, Cmat).real + x * Dskip[None, None, :]
        return y

    def _B_ref(x, w_gate, w_up, w_down):
        return (_gelu(x @ w_gate) * (x @ w_up)) @ w_down

    x = A_x
    xn = _layernorm(x, axis=-1)
    return x + _A_ref(xn, A_Lambda_re, A_Lambda_im, A_B_re, A_B_im, A_C_re, A_C_im, A_log_dt, A_Dskip) + _B_ref(xn, B_w_gate, B_w_up, B_w_down)
```

```python
import functools

import jax
import jax.numpy as jnp
import jax.experimental.pallas as pl
import jax.experimental.pallas.tpu as pltpu

_NSUB = 8


def _bf(v):
    return v.astype(jnp.bfloat16).astype(jnp.float32)


def _nt(a, b):
    return jax.lax.dot_general(a, b, (((1,), (1,)), ((), ())),
                               preferred_element_type=jnp.float32)


def _kernel(x_ref, lre_ref, lim_ref, ldt_ref, dsk_ref,
            bre_ref, bim_ref, cre_ref, cim_ref, wg_ref, wu_ref, wd_ref,
            o_ref,
            hre, him, pwre, pwim, par, st, *, tb, sc):
    step = pl.program_id(0)
    P = lre_ref.shape[1]

    @pl.when(step == 0)
    def _init():
        lre = lre_ref[...].astype(jnp.float32)
        lim = lim_ref[...].astype(jnp.float32)
        dt = _bf(jnp.exp(ldt_ref[...].astype(jnp.float32)))
        zr = dt * lre
        zi = dt * lim
        k = (jax.lax.broadcasted_iota(jnp.int32, (sc, P), 0) + 1).astype(jnp.float32)
        mag = jnp.exp(k * zr)
        pwre[...] = mag * jnp.cos(k * zi)
        pwim[...] = mag * jnp.sin(k * zi)
        are = pwre[0:1, :]
        aim = pwim[0:1, :]
        den = lre * lre + lim * lim
        nr = are - 1.0
        cre = (nr * lre + aim * lim) / den
        cim = (aim * lre - nr * lim) / den
        par[...] = jnp.concatenate(
            [are, aim, cre, cim, jnp.zeros((4, P), jnp.float32)], axis=0)
        st[...] = jnp.zeros(st.shape, jnp.float32)

    x = x_ref[...].astype(jnp.float32)
    m = _bf(jnp.mean(x, axis=-1, keepdims=True))
    mf = jnp.mean(x, axis=-1, keepdims=True)
    v = _bf(jnp.mean((x - mf) * (x - mf), axis=-1, keepdims=True))
    den = _bf(jnp.sqrt(_bf(v + 1e-5)))
    xn_f = _bf(_bf(x - m) / den)
    xn = xn_f.astype(jnp.bfloat16)

    are = par[0:1, :]
    aim = par[1:2, :]
    cr = par[2:3, :]
    ci = par[3:4, :]
    xbr = _nt(xn, bre_ref[...])
    xbi = _nt(xn, bim_ref[...])
    ncb = P // 128
    bur = cr * xbr - ci * xbi
    bui = cr * xbi + ci * xbr
    for c in range(ncb):
        hre[c] = bur[:, c * 128:(c + 1) * 128]
        him[c] = bui[:, c * 128:(c + 1) * 128]

    are8 = jnp.broadcast_to(are, (_NSUB, P))
    aim8 = jnp.broadcast_to(aim, (_NSUB, P))

    def body(t, carry):
        r, i = carry
        rows = pl.ds(t, _NSUB, stride=sc)
        br = jnp.concatenate([hre[c, rows, :] for c in range(ncb)], axis=1)
        bi = jnp.concatenate([him[c, rows, :] for c in range(ncb)], axis=1)
        nr_ = are8 * r - aim8 * i + br
        ni_ = are8 * i + aim8 * r + bi
        for c in range(ncb):
            hre[c, rows, :] = nr_[:, c * 128:(c + 1) * 128]
            him[c, rows, :] = ni_[:, c * 128:(c + 1) * 128]
        return nr_, ni_

    z8 = jnp.zeros((_NSUB, P), jnp.float32)
    er, ei = jax.lax.fori_loop(0, sc, body, (z8, z8), unroll=8)

    qr = pwre[sc - 1:sc, :]
    qi = pwim[sc - 1:sc, :]
    cr_ = st[0:1, :]
    ci_ = st[1:2, :]
    hr_l, hi_l = [], []
    for j in range(_NSUB):
        rows = pl.ds(j * sc, sc)
        pr = pwre[...]
        pi = pwim[...]
        lr = jnp.concatenate([hre[c, rows, :] for c in range(ncb)], axis=1)
        li = jnp.concatenate([him[c, rows, :] for c in range(ncb)], axis=1)
        hr_l.append((lr + pr * cr_ - pi * ci_).astype(jnp.bfloat16))
        hi_l.append((li + pr * ci_ + pi * cr_).astype(jnp.bfloat16))
        cr_, ci_ = (er[j:j + 1, :] + qr * cr_ - qi * ci_,
                    ei[j:j + 1, :] + qr * ci_ + qi * cr_)
    st[0:1, :] = cr_
    st[1:2, :] = ci_

    y = _nt(jnp.concatenate(hr_l, axis=0), cre_ref[...]) - _nt(
        jnp.concatenate(hi_l, axis=0), cim_ref[...])
    skip = _bf(xn_f * dsk_ref[...].astype(jnp.float32))

    g = _bf(jnp.dot(xn, wg_ref[...], preferred_element_type=jnp.float32))
    u = _bf(jnp.dot(xn, wu_ref[...], preferred_element_type=jnp.float32))
    hg = _bf(jax.nn.gelu(g, approximate=True))
    act = (hg * u).astype(jnp.bfloat16)
    f = _bf(jnp.dot(act, wd_ref[...], preferred_element_type=jnp.float32))

    o_ref[...] = x + (2.0 * y + skip) + f


@jax.jit
def pallas_parallel_sum__ssm_conv_s5__geglu_ffn__prompt_kernel(
    A_x: jax.Array,
    A_Lambda_re: jax.Array,
    A_Lambda_im: jax.Array,
    A_B_re: jax.Array,
    A_B_im: jax.Array,
    A_C_re: jax.Array,
    A_C_im: jax.Array,
    A_log_dt: jax.Array,
    A_Dskip: jax.Array,
    B_x: jax.Array,
    B_w_gate: jax.Array,
    B_w_up: jax.Array,
    B_w_down: jax.Array,
):
    Bsz, L, D = A_x.shape
    assert Bsz == 1
    P = A_Lambda_re.shape[0]
    F = B_w_gate.shape[1]
    tb = 512 if L % 512 == 0 else L
    sc = tb // _NSUB
    nb = L // tb

    x2 = A_x.reshape(L, D)
    row = lambda a: a.reshape(1, -1)
    const = lambda shape: pl.BlockSpec(shape, lambda i: (0, 0))

    out = pl.pallas_call(
        functools.partial(_kernel, tb=tb, sc=sc),
        grid=(nb,),
        in_specs=[
            pl.BlockSpec((tb, D), lambda i: (i, 0)),
            const((1, P)), const((1, P)), const((1, P)), const((1, D)),
            const((P, D)), const((P, D)), const((D, P)), const((D, P)),
            const((D, F)), const((D, F)), const((F, D)),
        ],
        out_specs=pl.BlockSpec((tb, D), lambda i: (i, 0)),
        out_shape=jax.ShapeDtypeStruct((L, D), jnp.float32),
        scratch_shapes=[
            pltpu.VMEM((P // 128, tb, 128), jnp.float32),
            pltpu.VMEM((P // 128, tb, 128), jnp.float32),
            pltpu.VMEM((sc, P), jnp.float32),
            pltpu.VMEM((sc, P), jnp.float32),
            pltpu.VMEM((8, P), jnp.float32),
            pltpu.VMEM((8, P), jnp.float32),
        ],
        compiler_params=pltpu.CompilerParams(
            dimension_semantics=("arbitrary",),
            vmem_limit_bytes=96 * 1024 * 1024,
        ),
    )(x2, row(A_Lambda_re), row(A_Lambda_im), row(A_log_dt), row(A_Dskip),
      A_B_re, A_B_im, A_C_re, A_C_im, B_w_gate, B_w_up, B_w_down)
    return out.reshape(Bsz, L, D)
```

```python
import functools

import jax
import jax.numpy as jnp
import jax.experimental.pallas as pl
import jax.experimental.pallas.tpu as pltpu

_NSUB = 8


def _bf(v):
    return v.astype(jnp.bfloat16).astype(jnp.float32)


def _nt(a, b):
    return jax.lax.dot_general(a, b, (((1,), (1,)), ((), ())),
                               preferred_element_type=jnp.float32)


def _kernel(x_ref, lre_ref, lim_ref, ldt_ref, dsk_ref,
            bre_hbm, bim_hbm, cre_hbm, cim_hbm, wg_hbm, wu_hbm, wd_hbm,
            o_ref,
            bre_ref, bim_ref, cre_ref, cim_ref, wg_ref, wu_ref, wd_ref, sems,
            hre, him, pwre, pwim, par, st, *, sc, pitch):
    step = pl.program_id(0)
    P = lre_ref.shape[0]
    ncb = P // 128

    srcs = (wg_hbm, wu_hbm, bre_hbm, bim_hbm, wd_hbm, cre_hbm, cim_hbm)
    dsts = (wg_ref, wu_ref, bre_ref, bim_ref, wd_ref, cre_ref, cim_ref)

    def copy(k):
        return pltpu.make_async_copy(srcs[k], dsts[k], sems.at[k])

    def row(ref):
        return ref[...].reshape(1, -1).astype(jnp.float32)

    def init():
        for k in range(len(srcs)):
            copy(k).start()
        lre = row(lre_ref)
        lim = row(lim_ref)
        dt = _bf(jnp.exp(row(ldt_ref)))
        zr = dt * lre
        zi = dt * lim
        k = (jax.lax.broadcasted_iota(jnp.int32, (sc, P), 0) + 1).astype(jnp.float32)
        mag = jnp.exp(k * zr)
        pwre[...] = mag * jnp.cos(k * zi)
        pwim[...] = mag * jnp.sin(k * zi)
        are = pwre[0:1, :]
        aim = pwim[0:1, :]
        den = lre * lre + lim * lim
        nr = are - 1.0
        cre = (nr * lre + aim * lim) / den
        cim = (aim * lre - nr * lim) / den
        par[...] = jnp.concatenate(
            [are, aim, cre, cim, row(dsk_ref), jnp.zeros((3, P), jnp.float32)], axis=0)
        st[...] = jnp.zeros(st.shape, jnp.float32)

    def body(first):
        def wait(*ks):
            if first:
                for k in ks:
                    copy(k).wait()

        tb = x_ref.shape[0]
        nq = 1 if first else 2
        xs, xns = [], []
        for q in range(nq):
            xq = x_ref[q * (tb // nq):(q + 1) * (tb // nq), :].astype(jnp.float32)
            mf = jnp.mean(xq, axis=-1, keepdims=True)
            m = _bf(mf)
            v = _bf(jnp.mean((xq - mf) * (xq - mf), axis=-1, keepdims=True))
            den = _bf(jnp.sqrt(_bf(v + 1e-5)))
            xns.append((_bf(xq - m) / den).astype(jnp.bfloat16))
            xs.append(xq)
        x = jnp.concatenate(xs, axis=0)
        xn = jnp.concatenate(xns, axis=0)
        xn_f = xn.astype(jnp.float32)

        def gate_up():
            wait(0)
            g = _bf(_nt(xn, wg_ref[...]))
            wait(1)
            return g, _bf(_nt(xn, wu_ref[...]))

        def down(g, u):
            hg = _bf(jax.nn.gelu(g, approximate=True))
            act = (hg * u).astype(jnp.bfloat16)
            wait(2, 3, 4)
            return _bf(jnp.dot(act, wd_ref[...], preferred_element_type=jnp.float32))

        if first:
            f = down(*gate_up())

        are = par[0:1, :]
        aim = par[1:2, :]
        cr = par[2:3, :]
        ci = par[3:4, :]
        xbr = jnp.concatenate([_nt(a, bre_ref[...]) for a in xns], axis=0)
        xbi = jnp.concatenate([_nt(a, bim_ref[...]) for a in xns], axis=0)
        bur = cr * xbr - ci * xbi
        bui = cr * xbi + ci * xbr
        for c in range(ncb):
            for j in range(_NSUB):
                hre[c, j * pitch:j * pitch + sc] = bur[j * sc:(j + 1) * sc, c * 128:(c + 1) * 128]
                him[c, j * pitch:j * pitch + sc] = bui[j * sc:(j + 1) * sc, c * 128:(c + 1) * 128]

        if not first:
            g, u = gate_up()

        are8 = jnp.broadcast_to(are, (_NSUB, P))
        aim8 = jnp.broadcast_to(aim, (_NSUB, P))
        er = jnp.zeros((_NSUB, P), jnp.float32)
        ei = er
        for t in range(sc):
            rows = pl.ds(t, _NSUB, stride=pitch)
            br = jnp.concatenate([hre[c, rows, :] for c in range(ncb)], axis=1)
            bi = jnp.concatenate([him[c, rows, :] for c in range(ncb)], axis=1)
            er, ei = are8 * er - aim8 * ei + br, are8 * ei + aim8 * er + bi
            for c in range(ncb):
                hre[c, rows, :] = er[:, c * 128:(c + 1) * 128]
                him[c, rows, :] = ei[:, c * 128:(c + 1) * 128]

        qr = pwre[sc - 1:sc, :]
        qi = pwim[sc - 1:sc, :]
        cr_ = st[0:1, :]
        ci_ = st[1:2, :]
        hr_l, hi_l = [], []
        for j in range(_NSUB):
            rows = pl.ds(j * pitch, sc)
            pr = pwre[...]
            pi = pwim[...]
            lr = jnp.concatenate([hre[c, rows, :] for c in range(ncb)], axis=1)
            li = jnp.concatenate([him[c, rows, :] for c in range(ncb)], axis=1)
            hr_l.append((lr + pr * cr_ - pi * ci_).astype(jnp.bfloat16))
            hi_l.append((li + pr * ci_ + pi * cr_).astype(jnp.bfloat16))
            cr_, ci_ = (er[j:j + 1, :] + qr * cr_ - qi * ci_,
                        ei[j:j + 1, :] + qr * ci_ + qi * cr_)
        st[0:1, :] = cr_
        st[1:2, :] = ci_

        wait(5, 6)
        y = _nt(jnp.concatenate(hr_l, axis=0), cre_ref[...]) - _nt(
            jnp.concatenate(hi_l, axis=0), cim_ref[...])
        skip = _bf(xn_f * par[4:5, :])
        if not first:
            f = down(g, u)

        o_ref[...] = x + (2.0 * y + skip) + f

    @pl.when(step == 0)
    def _():
        init()
        body(True)

    @pl.when(step > 0)
    def _():
        body(False)


@jax.jit
def pallas_parallel_sum__ssm_conv_s5__geglu_ffn__prompt_kernel(
    A_x: jax.Array,
    A_Lambda_re: jax.Array,
    A_Lambda_im: jax.Array,
    A_B_re: jax.Array,
    A_B_im: jax.Array,
    A_C_re: jax.Array,
    A_C_im: jax.Array,
    A_log_dt: jax.Array,
    A_Dskip: jax.Array,
    B_x: jax.Array,
    B_w_gate: jax.Array,
    B_w_up: jax.Array,
    B_w_down: jax.Array,
):
    Bsz, L, D = A_x.shape
    assert Bsz == 1
    P = A_Lambda_re.shape[0]
    F = B_w_gate.shape[1]
    assert P == D and P % 128 == 0 and L % (2 * _NSUB * 8) == 0
    tb = 512 if L % 512 == 0 else L
    sc = tb // _NSUB
    nb = L // tb
    pitch = sc + 4

    x2 = A_x.reshape(L, D)
    vec = lambda n: pl.BlockSpec((n,), lambda i: (0,))
    hbm = pl.BlockSpec(memory_space=pl.ANY)
    wdt = A_B_re.dtype

    out = pl.pallas_call(
        functools.partial(_kernel, sc=sc, pitch=pitch),
        grid=(nb,),
        in_specs=[
            pl.BlockSpec((tb, D), lambda i: (i, 0)),
            vec(P), vec(P), vec(P), vec(D),
            hbm, hbm, hbm, hbm, hbm, hbm, hbm,
        ],
        out_specs=pl.BlockSpec((tb, D), lambda i: (i, 0)),
        out_shape=jax.ShapeDtypeStruct((L, D), jnp.float32),
        scratch_shapes=[
            pltpu.VMEM((P, D), wdt),
            pltpu.VMEM((P, D), wdt),
            pltpu.VMEM((D, P), wdt),
            pltpu.VMEM((D, P), wdt),
            pltpu.VMEM((F, D), wdt),
            pltpu.VMEM((F, D), wdt),
            pltpu.VMEM((F, D), wdt),
            pltpu.SemaphoreType.DMA((7,)),
            pltpu.VMEM((P // 128, _NSUB * pitch, 128), jnp.float32),
            pltpu.VMEM((P // 128, _NSUB * pitch, 128), jnp.float32),
            pltpu.VMEM((sc, P), jnp.float32),
            pltpu.VMEM((sc, P), jnp.float32),
            pltpu.VMEM((8, P), jnp.float32),
            pltpu.VMEM((8, P), jnp.float32),
        ],
        compiler_params=pltpu.CompilerParams(
            dimension_semantics=("arbitrary",),
            vmem_limit_bytes=96 * 1024 * 1024,
        ),
    )(x2, A_Lambda_re, A_Lambda_im, A_log_dt, A_Dskip,
      A_B_re, A_B_im, A_C_re, A_C_im, B_w_gate.T, B_w_up.T, B_w_down)
    return out.reshape(Bsz, L, D)
```
